```python
import os as _os
_os.environ.setdefault("JAX_PLATFORMS", "cpu")
import jax
import jax.numpy as jnp

def _softmax(x, axis=-1):
    return jax.nn.softmax(x, axis=axis)
def _gelu(x):
    return jax.nn.gelu(x, approximate=True)
def _silu(x):
    return jax.nn.silu(x)
def _sigmoid(x):
    return jax.nn.sigmoid(x)
def _layernorm(x, axis=-1, eps=1e-5):
    m = jnp.mean(x, axis=axis, keepdims=True)
    v = jnp.var(x, axis=axis, keepdims=True)
    return (x - m) / jnp.sqrt(v + eps)
def _scatter_add(tgt, idx, src, axis=0):
    return tgt.at[idx].add(src)
def _segment_sum(src, seg, n):
    return jax.ops.segment_sum(src, seg, n)
class _Rng:
    def __init__(self, key):
        self._k = key
    def _next(self):
        self._k, sub = jax.random.split(self._k)
        return sub
    def normal(self, shape):
        return jax.random.normal(self._next(), shape, dtype=jnp.bfloat16)
    def randint(self, lo, hi, shape):
        return jax.random.randint(self._next(), shape, lo, hi, dtype=jnp.int32)
    def uniform(self, shape, lo=0.0, hi=1.0):
        return jax.random.uniform(self._next(), shape, jnp.bfloat16, lo, hi)
    def permutation(self, n):
        return jax.random.permutation(self._next(), n)


kernel_name = 'concat_heads__spectral_gfnet__sliding_block__prompt'

def setup_inputs():
    _rng = _Rng(jax.random.key(int.from_bytes(__import__("os").urandom(4), "little")))
    _w = (lambda a: (lambda t: t.astype(jnp.bfloat16) if jnp.issubdtype(t.dtype, jnp.floating) else t)(jnp.asarray(a)))
    def _A_setup():
        B, S, D = 1, 2048, 640
        Df = D // 2 + 1
        return {
            "x": _w((lambda *s: _rng.normal(s) * 0.05)(B, S, D)),
            "w_r": _w((lambda *s: _rng.normal(s) * 0.4)(S, Df) * 0.02),
            "w_i": _w((lambda *s: _rng.normal(s) * 0.4)(S, Df) * 0.02),
        }
    _A_in = _A_setup()

    def _B_setup():
        B, S, D = 1, 2048, 640
        return {
            "x": _w((lambda *s: _rng.normal(s) * 0.2)(B, S, D)),
            "wqkv": _w((lambda *s: _rng.normal(s) * 0.2)(D, 3 * D)),
            "wo": _w((lambda *s: _rng.normal(s) * 0.05)(D, D)),
        }
    _B_in = _B_setup()

    return {
        "A_x": _A_in["x"],
        "A_w_r": _A_in["w_r"],
        "A_w_i": _A_in["w_i"],
        "B_x": _B_in["x"],
        "B_wqkv": _B_in["wqkv"],
        "B_wo": _B_in["wo"],
    }

def reference(A_x, A_w_r, A_w_i, B_x, B_wqkv, B_wo):
    def _A_ref(x, w_r, w_i):
        B, S, D = x.shape
        X = (lambda x, axes=(-2,-1): jnp.fft.rfft2(x.astype(jnp.float32), axes=axes))(x, axes=(-2, -1))
        W = w_r + 1j * w_i
        X = X * W
        y = (lambda x, s, axes=(-2,-1): jnp.fft.irfft2(x, s=s, axes=axes).astype(jnp.bfloat16))(X, (S, D), axes=(-2, -1))
        return y

    def _B_ref(x, wqkv, wo):
        B, S, D = x.shape
        H = 32; Dh = D // H; W = 256
        qkv = (lambda x, *d: x.transpose(*d))((x @ wqkv).reshape(B, S, 3, H, Dh), 2, 0, 3, 1, 4)
        q, k, v = qkv[0], qkv[1], qkv[2]
        scores = jnp.einsum("bhqd,bhkd->bhqk", q, k) * (Dh ** -0.5)
        idx = jnp.arange(S)
        mask = (idx[:, None] - idx[None, :] >= 0) & (idx[:, None] - idx[None, :] < W)
        scores = jnp.where(mask[None, None], scores, -1e9)
        p = _softmax(scores, axis=-1)
        o = jnp.einsum("bhqk,bhkd->bhqd", p, v)
        return (lambda x, *d: x.transpose(*d))(o, 0, 2, 1, 3).reshape(B, S, D) @ wo

    a = _A_ref(A_x, A_w_r, A_w_i)
    b = _B_ref(B_x, B_wqkv, B_wo)
    return jnp.concatenate([a, b], axis=-1)
```

```python
import math

import numpy as np
import jax
import jax.numpy as jnp
from jax import lax
import jax.experimental.pallas as pl
import jax.experimental.pallas.tpu as pltpu

S = 2048
D = 640
DF = D // 2 + 1
FP = 384
H = 32
DH = 20
WIN = 256
BLK = 128
NB = S // BLK
KW = WIN + BLK

F32 = jnp.float32
BF16 = jnp.bfloat16


def _head_groups():
    groups = []
    for t in range(D // 128):
        full = [hh for hh in range(H)
                if (DH * hh) // 128 == t and (DH * hh + DH - 1) // 128 == t]
        groups.append((t, 128, full))
        strad = [hh for hh in range(H)
                 if (DH * hh) // 128 == t and (DH * hh + DH - 1) // 128 == t + 1]
        for hh in strad:
            groups.append((t, 256, [hh]))
    return groups


_GROUPS = _head_groups()


def _dft_tables():
    d = np.arange(D)[:, None]
    f = np.arange(DF)[None, :]
    ang = 2.0 * np.pi * ((d * f) % D) / D
    mf = np.zeros((D, 2 * FP), np.float64)
    mf[:, :DF] = np.cos(ang)
    mf[:, FP:FP + DF] = -np.sin(ang)
    c = np.full((DF,), 2.0)
    c[0] = 1.0
    c[DF - 1] = 1.0
    mi = np.zeros((2 * FP, D), np.float64)
    mi[:DF, :] = (c[:, None] * np.cos(ang.T)) / (D * S)
    mi[FP:FP + DF, :] = (-c[:, None] * np.sin(ang.T)) / (D * S)
    s1 = np.arange(BLK)
    k1 = np.arange(BLK)
    g = np.zeros((NB, 2 * BLK, BLK), np.float64)
    h = np.zeros((NB, 2 * BLK, BLK), np.float64)
    for k2 in range(NB):
        a = 2.0 * np.pi * ((s1[None, :] * (NB * k1[:, None] + k2)) % S) / S
        g[k2, :BLK] = np.cos(a)
        g[k2, BLK:] = -np.sin(a)
        h[k2, :BLK] = np.cos(a.T)
        h[k2, BLK:] = np.sin(a.T)
    return (mf, mi, g.reshape(NB * 2 * BLK, BLK), h.reshape(NB * 2 * BLK, BLK))


def _fft_list(re, im, sign):
    n = len(re)
    if n == 1:
        return re, im
    er, ei = _fft_list(re[0::2], im[0::2], sign)
    qr, qi = _fft_list(re[1::2], im[1::2], sign)
    outr = [None] * n
    outi = [None] * n
    for k in range(n // 2):
        xr, xi = qr[k], qi[k]
        if k == 0:
            tr, ti = xr, xi
        elif 4 * k == n:
            if sign > 0:
                tr, ti = -xi, xr
            else:
                tr, ti = xi, -xr
        elif 8 * k == n:
            c = math.sqrt(0.5)
            if sign > 0:
                tr, ti = (xr - xi) * c, (xi + xr) * c
            else:
                tr, ti = (xr + xi) * c, (xi - xr) * c
        elif 8 * k == 3 * n:
            c = math.sqrt(0.5)
            if sign > 0:
                tr, ti = (-xr - xi) * c, (xr - xi) * c
            else:
                tr, ti = (xi - xr) * c, (-xr - xi) * c
        else:
            ang = sign * 2.0 * math.pi * k / n
            c, s = math.cos(ang), math.sin(ang)
            tr = xr * c - xi * s
            ti = xr * s + xi * c
        outr[k] = er[k] + tr
        outi[k] = ei[k] + ti
        outr[k + n // 2] = er[k] - tr
        outi[k + n // 2] = ei[k] - ti
    return outr, outi


def _kernel(xa_h, wr_h, wi_h, xb_h, wqkv_h, wo_h, mf_h, mi_h, g_h, h_h, out_h,
            xa, wr, wi, xb, wqkv, wo, mf, mi, gm, hm,
            kscr, vtscr, otscr, qnext, knext, vtnext, wvt, wot, z, wfr, wfi, wtmp, ostage, astage, sems, osems):
    XB0 = 2 * BLK
    srcs = [wqkv_h, xb_h.at[pl.ds(0, XB0), :], wo_h, xa_h, mf_h, g_h, wr_h, wi_h, h_h, mi_h,
            xb_h.at[pl.ds(XB0, S - XB0), :]]
    dsts = [wqkv, xb.at[pl.ds(0, XB0), :], wo, xa, mf, gm, wr, wi, hm, mi,
            xb.at[pl.ds(XB0, S - XB0), :]]
    copies = [pltpu.make_async_copy(s_, d_, sems.at[n])
              for n, (s_, d_) in enumerate(zip(srcs, dsts))]
    for n in (0, 1, 2, 10, 3, 4, 5, 6, 7, 8, 9):
        copies[n].start()

    kscr[pl.ds(0, WIN), :] = jnp.zeros((WIN, D), BF16)
    vtscr[:, pl.ds(0, WIN)] = jnp.zeros((D, WIN), BF16)
    copies[0].wait()
    wvt[...] = wqkv[:, 2 * D:3 * D].astype(F32).T.astype(BF16)
    copies[1].wait()

    scale = DH ** -0.5 * math.log2(math.e)
    row = lax.broadcasted_iota(jnp.int32, (KW, BLK), 0)
    col = lax.broadcasted_iota(jnp.int32, (KW, BLK), 1)
    sub = lax.broadcasted_iota(jnp.int32, (8, BLK), 0)

    OCH = 256

    def out_copy(c, slot):
        return pltpu.make_async_copy(
            ostage.at[slot], out_h.at[pl.ds(c * OCH, OCH), pl.ds(D, D)], osems.at[slot])

    def proj_pieces(blk):
        rr = pl.multiple_of(blk * BLK, BLK)

        def qk_piece(t):
            def run():
                r = jnp.dot(xb[pl.ds(rr, BLK), :], wqkv[:, t * 128:(t + 1) * 128],
                            preferred_element_type=F32)
                if t < D // 128:
                    qnext[:, t * 128:(t + 1) * 128] = (r * scale).astype(BF16)
                else:
                    knext[:, t * 128 - D:(t + 1) * 128 - D] = r.astype(BF16)
            return run

        def v_piece(t):
            def run():
                r = lax.dot_general(wvt[t * 128:(t + 1) * 128, :], xb[pl.ds(rr, BLK), :],
                                    (((1,), (1,)), ((), ())), preferred_element_type=F32)
                vtnext[t * 128:(t + 1) * 128, :] = r.astype(BF16)
            return run

        return ([qk_piece(t) for t in range(2 * D // 128)]
                + [v_piece(t) for t in range(D // 128)])

    for run in proj_pieces(0):
        run()
    copies[2].wait()
    wot[...] = wo[...].astype(F32).T.astype(BF16)

    def qblock(i, carry):
        @pl.when(i == 1)
        def _():
            copies[10].wait()

        r0 = pl.multiple_of(i * BLK, BLK)
        q = qnext[...]
        kscr[pl.ds(r0 + WIN, BLK), :] = knext[...]
        vtscr[:, pl.ds(r0 + WIN, BLK)] = vtnext[...]
        todo = proj_pieces(jnp.minimum(i + 1, NB - 1))

        dist = col - row + WIN
        valid = jnp.logical_and(jnp.logical_and(dist >= 0, dist < WIN),
                                row + (i - 2) * BLK >= 0)
        bias = jnp.where(valid, 0.0, -1e30).astype(F32)

        def scores(grp):
            t0, w, heads = grp
            lane = lax.broadcasted_iota(jnp.int32, (BLK, w), 1) + t0 * 128
            qt = q[:, t0 * 128:t0 * 128 + w]
            qcat = jnp.concatenate(
                [jnp.where(jnp.logical_and(lane >= DH * hh, lane < DH * hh + DH),
                           qt, jnp.zeros((), BF16)) for hh in heads], axis=0)
            kt = kscr[pl.ds(r0, KW), t0 * 128:t0 * 128 + w]
            st = lax.dot_general(kt, qcat, (((1,), (1,)), ((), ())),
                                 preferred_element_type=F32)
            st = st + jnp.concatenate([bias] * len(heads), axis=1)
            return st, jnp.max(st, axis=0, keepdims=True)

        pieces = {}
        st_next = scores(_GROUPS[0])
        for gi, grp in enumerate(_GROUPS):
            st_all, m_all = st_next
            if gi + 1 < len(_GROUPS):
                st_next = scores(_GROUPS[gi + 1])
            for j, hh in enumerate(grp[2]):
                p = jnp.exp2(st_all[:, j * BLK:(j + 1) * BLK]
                             - m_all[:, j * BLK:(j + 1) * BLK])
                l = jnp.sum(p, axis=0, keepdims=True)
                a = ((DH * hh) // 16) * 16
                vth = vtscr[a:a + 32, pl.ds(r0, KW)]
                ot = jnp.dot(vth, p.astype(BF16), preferred_element_type=F32)
                pieces[hh] = ot * (1.0 / l)
                if hh % 2 == 1 and todo:
                    todo.pop(0)()
        rows = []
        for g in range(H // 4):
            o0, o1, o2, o3 = (pieces[4 * g + n] for n in range(4))
            rows += [o0[0:16], jnp.where(sub < 4, o0[16:24], o1[0:8]), o1[8:24],
                     o2[8:24], jnp.where(sub < 4, o2[24:32], o3[8:16]), o3[16:32]]
        otscr[:, pl.ds(r0, BLK)] = jnp.concatenate(rows, axis=0).astype(BF16)
        return carry

    with jax.named_scope('Bloop'):
        lax.fori_loop(0, NB, qblock, 0)

    with jax.named_scope('Bout'):
        for c in range(S // OCH):
            slot = c % 2
            if c >= 2:
                out_copy(c - 2, slot).wait()
            outt = jnp.dot(wot[...], otscr[:, pl.ds(c * OCH, OCH)], preferred_element_type=F32)
            ostage[slot] = outt.T.astype(BF16)
            out_copy(c, slot).start()

    for n in (3, 4, 5, 6, 7, 8, 9):
        copies[n].wait()

    with jax.named_scope('Wprep'):
        for src, dst in ((wr, wfr), (wi, wfi)):
            for j in range(2):
                dst[j] = src[pl.ds(128 * j, 128), :].astype(F32).T
            wtmp[...] = jnp.zeros((128, S), F32)
            wtmp[pl.ds(0, DF - 256), :] = src[pl.ds(256, DF - 256), :].astype(F32)
            dst[2] = wtmp[...].T

    CH = 256
    with jax.named_scope('A1'):
        for c in range(S // CH):
            z[pl.ds(c * CH, CH), :] = jnp.dot(xa[pl.ds(c * CH, CH), :], mf[...],
                                              preferred_element_type=F32)

    def radix16(sign):
        def body(g, carry):
            r0 = pl.multiple_of(g * 8, 8)
            for j in range(FP // 128):
                re = [z[pl.ds(r0 + BLK * b, 8), pl.ds(128 * j, 128)] for b in range(NB)]
                im = [z[pl.ds(r0 + BLK * b, 8), pl.ds(FP + 128 * j, 128)] for b in range(NB)]
                re, im = _fft_list(re, im, sign)
                for b in range(NB):
                    z[pl.ds(r0 + BLK * b, 8), pl.ds(128 * j, 128)] = re[b]
                    z[pl.ds(r0 + BLK * b, 8), pl.ds(FP + 128 * j, 128)] = im[b]
            return carry
        lax.fori_loop(0, BLK // 8, body, 0)

    with jax.named_scope('r16f'):
        radix16(-1)

    def mid(kk, carry):
        def fwd(k2):
            r0 = pl.multiple_of(k2 * BLK, BLK)
            g0 = pl.multiple_of(k2 * 2 * BLK, 2 * BLK)
            b = z[pl.ds(r0, BLK), :].astype(BF16)
            return jnp.dot(gm[pl.ds(g0, 2 * BLK), :], b, preferred_element_type=F32)

        def filt(k2, t):
            xr = t[:BLK, :FP] - t[BLK:, FP:]
            xi = t[:BLK, FP:] + t[BLK:, :FP]
            w_r = jnp.concatenate([wfr[j, pl.ds(k2, BLK, stride=NB), :] for j in range(3)], axis=1)
            w_i = jnp.concatenate([wfi[j, pl.ds(k2, BLK, stride=NB), :] for j in range(3)], axis=1)
            yr = xr * w_r - xi * w_i
            yi = xr * w_i + xi * w_r
            return jnp.concatenate([yr, yi], axis=1).astype(BF16)

        def inv(k2, y):
            r0 = pl.multiple_of(k2 * BLK, BLK)
            g0 = pl.multiple_of(k2 * 2 * BLK, 2 * BLK)
            t = jnp.dot(hm[pl.ds(g0, 2 * BLK), :], y, preferred_element_type=F32)
            z[pl.ds(r0, BLK), pl.ds(0, FP)] = t[:BLK, :FP] - t[BLK:, FP:]
            z[pl.ds(r0, BLK), pl.ds(FP, FP)] = t[:BLK, FP:] + t[BLK:, :FP]

        ks = [kk * MU + n for n in range(MU)]
        ts = [fwd(ks[0])]
        for n in range(MU):
            if n + 1 < MU:
                ts.append(fwd(ks[n + 1]))
            inv(ks[n], filt(ks[n], ts[n]))
        return carry

    MU = 4
    with jax.named_scope('mid'):
        lax.fori_loop(0, NB // MU, mid, 0)
    with jax.named_scope('r16i'):
        radix16(+1)

    def a_copy(c, slot):
        return pltpu.make_async_copy(
            astage.at[slot], out_h.at[pl.ds(c * CH, CH), pl.ds(0, D)], osems.at[2 + slot])

    nch = S // CH
    with jax.named_scope('A3'):
        for c in range(nch):
            slot = c % 2
            if c >= 2:
                a_copy(c - 2, slot).wait()
            astage[slot] = jnp.dot(z[pl.ds(c * CH, CH), :].astype(BF16), mi[...],
                                   preferred_element_type=F32).astype(BF16)
            a_copy(c, slot).start()
    a_copy(nch - 2, 0).wait()
    a_copy(nch - 1, 1).wait()
    out_copy(S // OCH - 2, 0).wait()
    out_copy(S // OCH - 1, 1).wait()


@jax.jit
def pallas_concat_heads__spectral_gfnet__sliding_block__prompt_kernel(
    A_x: jax.Array,
    A_w_r: jax.Array,
    A_w_i: jax.Array,
    B_x: jax.Array,
    B_wqkv: jax.Array,
    B_wo: jax.Array,
):
    mf, mi, g, h = (jnp.asarray(t, dtype=BF16) for t in _dft_tables())
    xa = A_x.reshape(S, D)
    xb = B_x.reshape(S, D)
    any_spec = pl.BlockSpec(memory_space=pl.ANY)
    out = pl.pallas_call(
        _kernel,
        out_shape=jax.ShapeDtypeStruct((S, 2 * D), BF16),
        in_specs=[any_spec] * 10,
        out_specs=any_spec,
        scratch_shapes=[
            pltpu.VMEM((S, D), BF16),
            pltpu.VMEM((DF, S), BF16),
            pltpu.VMEM((DF, S), BF16),
            pltpu.VMEM((S, D), BF16),
            pltpu.VMEM((D, 3 * D), BF16),
            pltpu.VMEM((D, D), BF16),
            pltpu.VMEM((D, 2 * FP), BF16),
            pltpu.VMEM((2 * FP, D), BF16),
            pltpu.VMEM((NB * 2 * BLK, BLK), BF16),
            pltpu.VMEM((NB * 2 * BLK, BLK), BF16),
            pltpu.VMEM((S + WIN, D), BF16),
            pltpu.VMEM((D, S + WIN), BF16),
            pltpu.VMEM((D, S), BF16),
            pltpu.VMEM((BLK, D), BF16),
            pltpu.VMEM((BLK, D), BF16),
            pltpu.VMEM((D, BLK), BF16),
            pltpu.VMEM((D, D), BF16),
            pltpu.VMEM((D, D), BF16),
            pltpu.VMEM((S, 2 * FP), F32),
            pltpu.VMEM((3, S, 128), F32),
            pltpu.VMEM((3, S, 128), F32),
            pltpu.VMEM((128, S), F32),
            pltpu.VMEM((2, 256, D), BF16),
            pltpu.VMEM((2, 256, D), BF16),
            pltpu.SemaphoreType.DMA((11,)),
            pltpu.SemaphoreType.DMA((4,)),
        ],
        compiler_params=pltpu.CompilerParams(vmem_limit_bytes=120 * 1024 * 1024),
    )(xa, A_w_r.T, A_w_i.T, xb, B_wqkv, B_wo, mf, mi, g, h)
    return out.reshape(1, S, 2 * D)
```

```python
import math

import numpy as np
import jax
import jax.numpy as jnp
from jax import lax
import jax.experimental.pallas as pl
import jax.experimental.pallas.tpu as pltpu

S = 2048
D = 640
DF = D // 2 + 1
FP = 384
H = 32
DH = 20
WIN = 256
BLK = 128
NB = S // BLK
KW = WIN + BLK

F32 = jnp.float32
BF16 = jnp.bfloat16


def _head_groups():
    groups = []
    for t in range(D // 128):
        full = [hh for hh in range(H)
                if (DH * hh) // 128 == t and (DH * hh + DH - 1) // 128 == t]
        groups.append((t, 128, full))
        strad = [hh for hh in range(H)
                 if (DH * hh) // 128 == t and (DH * hh + DH - 1) // 128 == t + 1]
        for hh in strad:
            groups.append((t, 256, [hh]))
    return groups


_GROUPS = _head_groups()


def _dft_tables():
    d1 = np.arange(128)[:, None]

    def cs(f2, n=64):
        a = 2.0 * np.pi * ((d1 * (5 * np.arange(n)[None, :] + f2)) % D) / D
        return np.cos(a), np.sin(a)

    mf = np.zeros((5 * 128, 256), np.float64)
    mi = np.zeros((6 * 128, 256), np.float64)
    nrm = 1.0 / (D * S)
    for n, (fa, fb) in enumerate(((1, 4), (2, 3))):
        ca, sa = cs(fa)
        cb, sb = cs(fb)
        m = mf[256 * n:256 * n + 256]
        m[:128, 0:64], m[128:, 0:64] = ca, sa
        m[:128, 64:128], m[128:, 64:128] = cb, -sb
        m[:128, 128:192], m[128:, 128:192] = -sa, ca
        m[:128, 192:256], m[128:, 192:256] = -sb, -cb
        v = mi[256 * n:256 * n + 256]
        v[0:64, :128], v[0:64, 128:] = 2 * nrm * ca.T, 2 * nrm * sa.T
        v[64:128, :128], v[64:128, 128:] = 2 * nrm * cb.T, -2 * nrm * sb.T
        v[128:192, :128], v[128:192, 128:] = -2 * nrm * sa.T, 2 * nrm * ca.T
        v[192:256, :128], v[192:256, 128:] = -2 * nrm * sb.T, -2 * nrm * cb.T
    c0, s0 = cs(0, 65)
    mf[512:640, 0:65] = c0
    mf[512:640, 128:193] = -s0
    wt = np.full((65, 1), 2.0 * nrm)
    wt[0] = nrm
    wt[64] = nrm
    mi[512:577, :128] = wt * c0.T
    mi[640:705, :128] = -wt * s0.T
    s1 = np.arange(BLK)
    k1 = np.arange(BLK)
    g = np.zeros((NB, 3 * BLK, BLK), np.float64)
    h = np.zeros((NB, 3 * BLK, BLK), np.float64)
    for k2 in range(NB):
        a = 2.0 * np.pi * ((s1[None, :] * (NB * k1[:, None] + k2)) % S) / S
        g[k2, :BLK] = np.cos(a)
        g[k2, BLK:2 * BLK] = -np.sin(a)
        g[k2, 2 * BLK:] = np.cos(a) - np.sin(a)
        h[k2, :BLK] = np.cos(a.T)
        h[k2, BLK:2 * BLK] = np.sin(a.T)
        h[k2, 2 * BLK:] = np.cos(a.T) + np.sin(a.T)
    return (mf, mi, g.reshape(NB * 3 * BLK, BLK), h.reshape(NB * 3 * BLK, BLK))


def _fft_list(re, im, sign):
    n = len(re)
    if n == 1:
        return re, im
    er, ei = _fft_list(re[0::2], im[0::2], sign)
    qr, qi = _fft_list(re[1::2], im[1::2], sign)
    outr = [None] * n
    outi = [None] * n
    for k in range(n // 2):
        xr, xi = qr[k], qi[k]
        if k == 0:
            tr, ti = xr, xi
        elif 4 * k == n:
            if sign > 0:
                tr, ti = -xi, xr
            else:
                tr, ti = xi, -xr
        elif 8 * k == n:
            c = math.sqrt(0.5)
            if sign > 0:
                tr, ti = (xr - xi) * c, (xi + xr) * c
            else:
                tr, ti = (xr + xi) * c, (xi - xr) * c
        elif 8 * k == 3 * n:
            c = math.sqrt(0.5)
            if sign > 0:
                tr, ti = (-xr - xi) * c, (xr - xi) * c
            else:
                tr, ti = (xi - xr) * c, (-xr - xi) * c
        else:
            ang = sign * 2.0 * math.pi * k / n
            c, s = math.cos(ang), math.sin(ang)
            tr = xr * c - xi * s
            ti = xr * s + xi * c
        outr[k] = er[k] + tr
        outi[k] = ei[k] + ti
        outr[k + n // 2] = er[k] - tr
        outi[k + n // 2] = ei[k] - ti
    return outr, outi


def _kernel(xa_h, wr_h, wi_h, xb_h, wqkv_h, wo_h, mf_h, mi_h, g_h, h_h, out_h,
            xa, wr, wi, xb, wqkv, wo, mf, mi, gm, hm,
            kscr, vtscr, otscr, qnext, knext, vtnext, wvt, wot, z, wfr, wfi, wtr, wti,
            ostage, astage, sems, xsems, osems):
    XB0 = 2 * BLK
    CH = 256
    NCH = S // CH
    srcs = [wqkv_h.at[:, pl.ds(0, D)], xb_h.at[pl.ds(0, XB0), :], wo_h, mf_h, g_h, wr_h, wi_h,
            h_h, mi_h, xb_h.at[pl.ds(XB0, S - XB0), :],
            wqkv_h.at[:, pl.ds(D, D)], wqkv_h.at[:, pl.ds(2 * D, D)]]
    dsts = [wqkv.at[:, pl.ds(0, D)], xb.at[pl.ds(0, XB0), :], wo, mf, gm, wr, wi,
            hm, mi, xb.at[pl.ds(XB0, S - XB0), :],
            wqkv.at[:, pl.ds(D, D)], wqkv.at[:, pl.ds(2 * D, D)]]
    copies = [pltpu.make_async_copy(s_, d_, sems.at[n])
              for n, (s_, d_) in enumerate(zip(srcs, dsts))]

    def xa_copy(c):
        rows = pl.ds(pl.multiple_of(c * CH, CH), CH)
        return pltpu.make_async_copy(xa_h.at[rows, :], xa.at[rows, :], xsems.at[c])

    for n in (1, 0, 10, 11, 3):
        copies[n].start()
    xa_copy(0).start()
    for n in (9, 2):
        copies[n].start()
    for c in range(1, NCH):
        xa_copy(c).start()
    for n in (4, 5, 6, 7, 8):
        copies[n].start()

    scale = DH ** -0.5 * math.log2(math.e)
    sub = lax.broadcasted_iota(jnp.int32, (8, BLK), 0)
    C1, S1 = math.cos(2 * math.pi / 5), math.sin(2 * math.pi / 5)
    C2, S2 = math.cos(4 * math.pi / 5), math.sin(4 * math.pi / 5)

    def out_copy(c):
        return pltpu.make_async_copy(
            ostage.at[pl.ds(c * CH, CH), :], out_h.at[pl.ds(c * CH, CH), pl.ds(D, D)],
            osems.at[c])

    def proj_pieces(blk):
        rr = pl.multiple_of(blk * BLK, BLK)

        def qk_piece(t):
            def run():
                r = jnp.dot(xb[pl.ds(rr, BLK), :], wqkv[:, t * 128:(t + 1) * 128],
                            preferred_element_type=F32)
                if t < D // 128:
                    qnext[:, t * 128:(t + 1) * 128] = (r * scale).astype(BF16)
                else:
                    knext[:, t * 128 - D:(t + 1) * 128 - D] = r.astype(BF16)
            return run

        def v_piece(t):
            def run():
                r = lax.dot_general(wvt[t * 128:(t + 1) * 128, :], xb[pl.ds(rr, BLK), :],
                                    (((1,), (1,)), ((), ())), preferred_element_type=F32)
                vtnext[t * 128:(t + 1) * 128, :] = r.astype(BF16)
            return run

        return ([qk_piece(t) for t in range(2 * D // 128)]
                + [v_piece(t) for t in range(D // 128)])

    def bout_piece(c):
        outt = jnp.dot(wot[...], otscr[:, pl.ds(c * BLK, BLK)], preferred_element_type=F32)
        ostage[pl.ds(c * BLK, BLK), :] = outt.T.astype(BF16)
        if c % 2 == 1:
            out_copy(c // 2).start()

    def a1_pieces(c):
        rows = pl.ds(pl.multiple_of(c * CH, CH), CH)
        st = {}

        def prep():
            x0, x1, x2, x3, x4 = (xa[rows, pl.ds(128 * n, 128)].astype(F32) for n in range(5))
            a1, a2, b1, b2 = x1 + x4, x2 + x3, x1 - x4, x2 - x3
            st[2] = (x0 + a1 + a2).astype(BF16)
            st[0] = jnp.concatenate([x0 + C1 * a1 + C2 * a2, -(S1 * b1 + S2 * b2)],
                                    axis=1).astype(BF16)
            st[1] = jnp.concatenate([x0 + C2 * a1 + C1 * a2, S1 * b2 - S2 * b1],
                                    axis=1).astype(BF16)

        def mm(n):
            def run():
                u = st[n]
                r = jnp.dot(u, mf[pl.ds(256 * n, u.shape[1]), :], preferred_element_type=F32)
                z[rows, pl.ds(128 * n, 128)] = r[:, :128]
                z[rows, pl.ds(FP + 128 * n, 128)] = r[:, 128:]
            return run

        return [prep, mm(0), mm(1), mm(2)]

    def mid_pieces(k2):
        r0 = pl.multiple_of(k2 * BLK, BLK)
        g0 = pl.multiple_of(k2 * 3 * BLK, BLK)
        st = {}

        def cmul(tab, br, bi):
            t1 = jnp.dot(tab[pl.ds(g0, BLK), :], br.astype(BF16), preferred_element_type=F32)
            t2 = jnp.dot(tab[pl.ds(g0 + BLK, BLK), :], bi.astype(BF16),
                         preferred_element_type=F32)
            t3 = jnp.dot(tab[pl.ds(g0 + 2 * BLK, BLK), :], (br + bi).astype(BF16),
                         preferred_element_type=F32)
            return t1 - t2, t3 - t1 - t2

        def fwd():
            st[0] = cmul(gm, z[pl.ds(r0, BLK), pl.ds(0, FP)], z[pl.ds(r0, BLK), pl.ds(FP, FP)])

        def inv():
            xr, xi = st[0]
            w_r = jnp.concatenate([wfr[j, pl.ds(k2, BLK, stride=NB), :] for j in range(3)], axis=1)
            w_i = jnp.concatenate([wfi[j, pl.ds(k2, BLK, stride=NB), :] for j in range(3)], axis=1)
            yr = xr * w_r - xi * w_i
            yi = xr * w_i + xi * w_r
            ur, ui = cmul(hm, yr, yi)
            z[pl.ds(r0, BLK), pl.ds(0, FP)] = ur
            z[pl.ds(r0, BLK), pl.ds(FP, FP)] = ui

        return [fwd, inv]

    def wprep_load(n):
        src, dst = ((wr, wtr), (wi, wti))[n]
        for b in range(NB):
            dst[b, pl.ds(320, 8), :] = jnp.zeros((8, 128), F32)
            dst[b, pl.ds(0, DF), :] = src[:, pl.ds(BLK * b, BLK)].astype(F32)

    def wprep_piece(n):
        src, dst = ((wtr, wfr), (wti, wfi))[n // 4]
        for b in range(4 * (n % 4), 4 * (n % 4) + 4):
            rows = [src[b, pl.ds(f2, 64, stride=5), :] for f2 in range(5)]
            dst[0, pl.ds(BLK * b, BLK), :] = jnp.concatenate([rows[1], rows[4]], axis=0).T
            dst[1, pl.ds(BLK * b, BLK), :] = jnp.concatenate([rows[2], rows[3]], axis=0).T
            last = jnp.where(sub == 0, src[b, pl.ds(320, 8), :], 0.0)
            dst[2, pl.ds(BLK * b, BLK), :] = jnp.concatenate(
                [rows[0], last, jnp.zeros((56, 128), F32)], axis=0).T

    def radix16_piece(sign, g, j):
        r0 = g * 8
        re = [z[pl.ds(r0 + BLK * b, 8), pl.ds(128 * j, 128)] for b in range(NB)]
        im = [z[pl.ds(r0 + BLK * b, 8), pl.ds(FP + 128 * j, 128)] for b in range(NB)]
        re, im = _fft_list(re, im, sign)
        for b in range(NB):
            z[pl.ds(r0 + BLK * b, 8), pl.ds(128 * j, 128)] = re[b]
            z[pl.ds(r0 + BLK * b, 8), pl.ds(FP + 128 * j, 128)] = im[b]

    def radix16(sign, bouts, extra):
        n = 0
        for g in range(BLK // 8):
            for j in range(FP // 128):
                if n % 6 == 0 and bouts:
                    bout_piece(bouts.pop(0))
                if n % 6 == 3 and extra:
                    wprep_piece(extra.pop(0))
                radix16_piece(sign, g, j)
                n += 1

    def make_qblock(first_half, kw=KW, last=False):
        koff = KW - kw
        row = lax.broadcasted_iota(jnp.int32, (kw, BLK), 0) + koff
        col = lax.broadcasted_iota(jnp.int32, (kw, BLK), 1)

        def qblock(i, carry):
            if first_half:
                xa_copy(i).wait()
                extra = a1_pieces(i)
            else:
                ma = mid_pieces(2 * (i - NB // 2))
                mb = mid_pieces(2 * (i - NB // 2) + 1)
                extra = [ma[0], mb[0], ma[1], mb[1]]

            r0 = pl.multiple_of(i * BLK, BLK)
            q = qnext[...]
            kscr[pl.ds(r0 + WIN, BLK), :] = knext[...]
            vtscr[:, pl.ds(r0 + WIN, BLK)] = vtnext[...]
            todo = [] if last else proj_pieces(i + 1)

            dist = col - row + WIN
            valid = jnp.logical_and(dist >= 0, dist < WIN)
            bias = jnp.where(valid, 0.0, -1e30).astype(F32)

            def scores(grp):
                t0, w, heads = grp
                lane = lax.broadcasted_iota(jnp.int32, (BLK, w), 1) + t0 * 128
                qt = q[:, t0 * 128:t0 * 128 + w]
                qcat = jnp.concatenate(
                    [jnp.where(jnp.logical_and(lane >= DH * hh, lane < DH * hh + DH),
                               qt, jnp.zeros((), BF16)) for hh in heads], axis=0)
                kt = kscr[pl.ds(r0 + koff, kw), t0 * 128:t0 * 128 + w]
                st = lax.dot_general(kt, qcat, (((1,), (1,)), ((), ())),
                                     preferred_element_type=F32)
                bcat = jnp.concatenate([bias] * len(heads), axis=1)
                if kw < KW:
                    st = st + bcat
                else:
                    st = jnp.concatenate(
                        [st[:BLK] + bcat[:BLK], st[BLK:2 * BLK],
                         st[2 * BLK:] + bcat[2 * BLK:]], axis=0)
                return st, jnp.max(st, axis=0, keepdims=True)

            pieces = {}
            st_next = scores(_GROUPS[0])
            for gi, grp in enumerate(_GROUPS):
                st_all, m_all = st_next
                if gi + 1 < len(_GROUPS):
                    st_next = scores(_GROUPS[gi + 1])
                for j, hh in enumerate(grp[2]):
                    p = jnp.exp2(st_all[:, j * BLK:(j + 1) * BLK]
                                 - m_all[:, j * BLK:(j + 1) * BLK])
                    l = jnp.sum(p, axis=0, keepdims=True)
                    a = ((DH * hh) // 16) * 16
                    vth = vtscr[a:a + 32, pl.ds(r0 + koff, kw)]
                    ot = jnp.dot(vth, p.astype(BF16), preferred_element_type=F32)
                    pieces[hh] = ot * (1.0 / l)
                    if hh % 2 == 1 and todo:
                        todo.pop(0)()
                    if hh % 6 == 2 and extra:
                        extra.pop(0)()
            while todo:
                todo.pop(0)()
            while extra:
                extra.pop(0)()
            rows = []
            for g in range(H // 4):
                o0, o1, o2, o3 = (pieces[4 * g + n] for n in range(4))
                rows += [o0[0:16], jnp.where(sub < 4, o0[16:24], o1[0:8]), o1[8:24],
                         o2[8:24], jnp.where(sub < 4, o2[24:32], o3[8:16]), o3[16:32]]
            otscr[:, pl.ds(r0, BLK)] = jnp.concatenate(rows, axis=0).astype(BF16)
            return carry
        return qblock

    first = proj_pieces(0)
    copies[1].wait()
    copies[0].wait()
    for run in first[:5]:
        run()
    copies[10].wait()
    for run in first[5:10]:
        run()
    copies[11].wait()
    wvt[...] = wqkv[:, 2 * D:3 * D].astype(F32).T.astype(BF16)
    for run in first[10:]:
        run()
    copies[3].wait()

    with jax.named_scope('loop1'):
        make_qblock(True, BLK)(0, 0)
        copies[9].wait()
        make_qblock(True, 2 * BLK)(1, 0)
        lax.fori_loop(2, NB // 2, make_qblock(True), 0)

    for n in (2, 4, 5, 6, 7, 8):
        copies[n].wait()
    with jax.named_scope('r16f'):
        wot[...] = wo[...].astype(F32).T.astype(BF16)
        wprep_load(0)
        wprep_load(1)
        radix16(-1, list(range(0, NB // 2)), list(range(8)))

    with jax.named_scope('loop2'):
        lax.fori_loop(NB // 2, NB - 1, make_qblock(False), 0)
        make_qblock(False, last=True)(NB - 1, 0)

    with jax.named_scope('r16i'):
        radix16(+1, list(range(NB // 2, NB)), [])

    def a_copy(c):
        return pltpu.make_async_copy(
            astage.at[pl.ds(c * CH, CH), :], out_h.at[pl.ds(c * CH, CH), pl.ds(0, D)],
            osems.at[NCH + c])

    with jax.named_scope('A3'):
        for c in range(NCH):
            rows = pl.ds(c * CH, CH)
            t = []
            for n in range(3):
                y = jnp.concatenate([z[rows, pl.ds(128 * n, 128)],
                                     z[rows, pl.ds(FP + 128 * n, 128)]], axis=1).astype(BF16)
                if n < 2:
                    t.append(jnp.dot(y, mi[pl.ds(256 * n, 256), :], preferred_element_type=F32))
                else:
                    t.append(jnp.dot(y, mi[pl.ds(512, 256), pl.ds(0, 128)],
                                     preferred_element_type=F32))
            p1, q1 = t[0][:, :128], t[0][:, 128:]
            p2, q2 = t[1][:, :128], t[1][:, 128:]
            t0 = t[2]
            e1, o1 = t0 + C1 * p1 + C2 * p2, S1 * q1 + S2 * q2
            e2, o2 = t0 + C2 * p1 + C1 * p2, S2 * q1 - S1 * q2
            astage[rows, :] = jnp.concatenate(
                [t0 + p1 + p2, e1 - o1, e2 - o2, e2 + o2, e1 + o1], axis=1).astype(BF16)
            a_copy(c).start()
    for c in range(NCH):
        out_copy(c).wait()
        a_copy(c).wait()


@jax.jit
def pallas_concat_heads__spectral_gfnet__sliding_block__prompt_kernel(
    A_x: jax.Array,
    A_w_r: jax.Array,
    A_w_i: jax.Array,
    B_x: jax.Array,
    B_wqkv: jax.Array,
    B_wo: jax.Array,
):
    mf, mi, g, h = (jnp.asarray(t, dtype=BF16) for t in _dft_tables())
    xa = A_x.reshape(S, D)
    xb = B_x.reshape(S, D)
    any_spec = pl.BlockSpec(memory_space=pl.ANY)
    out = pl.pallas_call(
        _kernel,
        out_shape=jax.ShapeDtypeStruct((S, 2 * D), BF16),
        in_specs=[any_spec] * 10,
        out_specs=any_spec,
        scratch_shapes=[
            pltpu.VMEM((S, D), BF16),
            pltpu.VMEM((DF, S), BF16),
            pltpu.VMEM((DF, S), BF16),
            pltpu.VMEM((S, D), BF16),
            pltpu.VMEM((D, 3 * D), BF16),
            pltpu.VMEM((D, D), BF16),
            pltpu.VMEM((5 * 128, 256), BF16),
            pltpu.VMEM((6 * 128, 256), BF16),
            pltpu.VMEM((NB * 3 * BLK, BLK), BF16),
            pltpu.VMEM((NB * 3 * BLK, BLK), BF16),
            pltpu.VMEM((S + WIN, D), BF16),
            pltpu.VMEM((D, S + WIN), BF16),
            pltpu.VMEM((D, S), BF16),
            pltpu.VMEM((BLK, D), BF16),
            pltpu.VMEM((BLK, D), BF16),
            pltpu.VMEM((D, BLK), BF16),
            pltpu.VMEM((D, D), BF16),
            pltpu.VMEM((D, D), BF16),
            pltpu.VMEM((S, 2 * FP), F32),
            pltpu.VMEM((3, S, 128), F32),
            pltpu.VMEM((3, S, 128), F32),
            pltpu.VMEM((NB, 328, 128), F32),
            pltpu.VMEM((NB, 328, 128), F32),
            pltpu.VMEM((S, D), BF16),
            pltpu.VMEM((S, D), BF16),
            pltpu.SemaphoreType.DMA((12,)),
            pltpu.SemaphoreType.DMA((8,)),
            pltpu.SemaphoreType.DMA((16,)),
        ],
        compiler_params=pltpu.CompilerParams(vmem_limit_bytes=120 * 1024 * 1024),
    )(xa, A_w_r.T, A_w_i.T, xb, B_wqkv, B_wo, mf, mi, g, h)
    return out.reshape(1, S, 2 * D)
```

```python
import math

import numpy as np
import jax
import jax.numpy as jnp
from jax import lax
import jax.experimental.pallas as pl
import jax.experimental.pallas.tpu as pltpu

S = 2048
D = 640
DF = D // 2 + 1
FP = 384
H = 32
DH = 20
WIN = 256
BLK = 128
NB = S // BLK
KW = WIN + BLK

F32 = jnp.float32
BF16 = jnp.bfloat16


def _head_groups():
    groups = []
    for t in range(D // 128):
        full = [hh for hh in range(H)
                if (DH * hh) // 128 == t and (DH * hh + DH - 1) // 128 == t]
        groups.append((t, 128, full))
        strad = [hh for hh in range(H)
                 if (DH * hh) // 128 == t and (DH * hh + DH - 1) // 128 == t + 1]
        for hh in strad:
            groups.append((t, 256, [hh]))
    return groups


_GROUPS = _head_groups()


def _dft_tables():
    d1 = np.arange(128)[:, None]

    def cs(f2, n=64):
        a = 2.0 * np.pi * ((d1 * (5 * np.arange(n)[None, :] + f2)) % D) / D
        return np.cos(a), np.sin(a)

    mf = np.zeros((5 * 128, 256), np.float64)
    mi = np.zeros((6 * 128, 256), np.float64)
    nrm = 1.0 / (D * S)
    for n, (fa, fb) in enumerate(((1, 4), (2, 3))):
        ca, sa = cs(fa)
        cb, sb = cs(fb)
        m = mf[256 * n:256 * n + 256]
        m[:128, 0:64], m[128:, 0:64] = ca, sa
        m[:128, 64:128], m[128:, 64:128] = cb, -sb
        m[:128, 128:192], m[128:, 128:192] = -sa, ca
        m[:128, 192:256], m[128:, 192:256] = -sb, -cb
        v = mi[256 * n:256 * n + 256]
        v[0:64, :128], v[0:64, 128:] = 2 * nrm * ca.T, 2 * nrm * sa.T
        v[64:128, :128], v[64:128, 128:] = 2 * nrm * cb.T, -2 * nrm * sb.T
        v[128:192, :128], v[128:192, 128:] = -2 * nrm * sa.T, 2 * nrm * ca.T
        v[192:256, :128], v[192:256, 128:] = -2 * nrm * sb.T, -2 * nrm * cb.T
    c0, s0 = cs(0, 65)
    mf[512:640, 0:65] = c0
    mf[512:640, 128:193] = -s0
    wt = np.full((65, 1), 2.0 * nrm)
    wt[0] = nrm
    wt[64] = nrm
    mi[512:577, :128] = wt * c0.T
    mi[640:705, :128] = -wt * s0.T
    s1 = np.arange(BLK)
    k1 = np.arange(BLK)
    g = np.zeros((NB, 3 * BLK, BLK), np.float64)
    h = np.zeros((NB, 3 * BLK, BLK), np.float64)
    for k2 in range(NB):
        a = 2.0 * np.pi * ((s1[None, :] * (NB * k1[:, None] + k2)) % S) / S
        g[k2, :BLK] = np.cos(a)
        g[k2, BLK:2 * BLK] = -np.sin(a)
        g[k2, 2 * BLK:] = np.cos(a) - np.sin(a)
        h[k2, :BLK] = np.cos(a.T)
        h[k2, BLK:2 * BLK] = np.sin(a.T)
        h[k2, 2 * BLK:] = np.cos(a.T) + np.sin(a.T)
    return (mf, mi, g.reshape(NB * 3 * BLK, BLK), h.reshape(NB * 3 * BLK, BLK))


def _fft_list(re, im, sign):
    n = len(re)
    if n == 1:
        return re, im
    er, ei = _fft_list(re[0::2], im[0::2], sign)
    qr, qi = _fft_list(re[1::2], im[1::2], sign)
    outr = [None] * n
    outi = [None] * n
    for k in range(n // 2):
        xr, xi = qr[k], qi[k]
        if k == 0:
            tr, ti = xr, xi
        elif 4 * k == n:
            if sign > 0:
                tr, ti = -xi, xr
            else:
                tr, ti = xi, -xr
        elif 8 * k == n:
            c = math.sqrt(0.5)
            if sign > 0:
                tr, ti = (xr - xi) * c, (xi + xr) * c
            else:
                tr, ti = (xr + xi) * c, (xi - xr) * c
        elif 8 * k == 3 * n:
            c = math.sqrt(0.5)
            if sign > 0:
                tr, ti = (-xr - xi) * c, (xr - xi) * c
            else:
                tr, ti = (xi - xr) * c, (-xr - xi) * c
        else:
            ang = sign * 2.0 * math.pi * k / n
            c, s = math.cos(ang), math.sin(ang)
            tr = xr * c - xi * s
            ti = xr * s + xi * c
        outr[k] = er[k] + tr
        outi[k] = ei[k] + ti
        outr[k + n // 2] = er[k] - tr
        outi[k + n // 2] = ei[k] - ti
    return outr, outi


def _kernel(xa_h, wr_h, wi_h, xb_h, wqkv_h, wo_h, mf_h, mi_h, g_h, h_h, out_h,
            xa, wr, wi, xb, wqkv, wo, mf, mi, gm, hm,
            kscr, vtscr, otscr, qnext, knext, vtnext, wvt, z, wfr, wfi, wtr, wti,
            ostage, astage, sems, xsems, osems):
    XB0 = 2 * BLK
    CH = 256
    NCH = S // CH
    srcs = [wqkv_h.at[:, pl.ds(0, D)], xb_h.at[pl.ds(0, XB0), :], wo_h, mf_h, g_h, wr_h, wi_h,
            h_h, mi_h, xb_h.at[pl.ds(XB0, S - XB0), :],
            wqkv_h.at[:, pl.ds(D, D)], wqkv_h.at[:, pl.ds(2 * D, D)]]
    dsts = [wqkv.at[:, pl.ds(0, D)], xb.at[pl.ds(0, XB0), :], wo, mf, gm, wr, wi,
            hm, mi, xb.at[pl.ds(XB0, S - XB0), :],
            wqkv.at[:, pl.ds(D, D)], wqkv.at[:, pl.ds(2 * D, D)]]
    copies = [pltpu.make_async_copy(s_, d_, sems.at[n])
              for n, (s_, d_) in enumerate(zip(srcs, dsts))]

    def xa_copy(c):
        rows = pl.ds(pl.multiple_of(c * CH, CH), CH)
        return pltpu.make_async_copy(xa_h.at[rows, :], xa.at[rows, :], xsems.at[c])

    for n in (1, 0, 10, 11, 3):
        copies[n].start()
    xa_copy(0).start()
    for n in (9, 2):
        copies[n].start()
    for c in range(1, NCH):
        xa_copy(c).start()
    for n in (4, 5, 6, 7, 8):
        copies[n].start()

    scale = DH ** -0.5 * math.log2(math.e)
    sub = lax.broadcasted_iota(jnp.int32, (8, BLK), 0)
    C1, S1 = math.cos(2 * math.pi / 5), math.sin(2 * math.pi / 5)
    C2, S2 = math.cos(4 * math.pi / 5), math.sin(4 * math.pi / 5)

    def out_copy(c):
        return pltpu.make_async_copy(
            ostage.at[pl.ds(c * CH, CH), :], out_h.at[pl.ds(c * CH, CH), pl.ds(D, D)],
            osems.at[c])

    def proj_pieces(blk):
        rr = pl.multiple_of(blk * BLK, BLK)

        def qk_piece(t):
            def run():
                r = jnp.dot(xb[pl.ds(rr, BLK), :], wqkv[:, t * 128:(t + 1) * 128],
                            preferred_element_type=F32)
                if t < D // 128:
                    qnext[:, t * 128:(t + 1) * 128] = (r * scale).astype(BF16)
                else:
                    knext[:, t * 128 - D:(t + 1) * 128 - D] = r.astype(BF16)
            return run

        def v_piece(t):
            def run():
                r = lax.dot_general(wvt[t * 128:(t + 1) * 128, :], xb[pl.ds(rr, BLK), :],
                                    (((1,), (1,)), ((), ())), preferred_element_type=F32)
                vtnext[t * 128:(t + 1) * 128, :] = r.astype(BF16)
            return run

        return ([qk_piece(t) for t in range(2 * D // 128)]
                + [v_piece(t) for t in range(D // 128)])

    def bout_piece(c):
        outb = lax.dot_general(otscr[:, pl.ds(c * BLK, BLK)], wo[...],
                               (((0,), (0,)), ((), ())), preferred_element_type=F32)
        ostage[pl.ds(c * BLK, BLK), :] = outb.astype(BF16)
        if c % 2 == 1:
            out_copy(c // 2).start()

    def a1_pieces(c):
        rows = pl.ds(pl.multiple_of(c * CH, CH), CH)
        st = {}

        def prep():
            x0, x1, x2, x3, x4 = (xa[rows, pl.ds(128 * n, 128)].astype(F32) for n in range(5))
            a1, a2, b1, b2 = x1 + x4, x2 + x3, x1 - x4, x2 - x3
            st[2] = (x0 + a1 + a2).astype(BF16)
            st[0] = jnp.concatenate([x0 + C1 * a1 + C2 * a2, -(S1 * b1 + S2 * b2)],
                                    axis=1).astype(BF16)
            st[1] = jnp.concatenate([x0 + C2 * a1 + C1 * a2, S1 * b2 - S2 * b1],
                                    axis=1).astype(BF16)

        def mm(n):
            def run():
                u = st[n]
                r = jnp.dot(u, mf[pl.ds(256 * n, u.shape[1]), :], preferred_element_type=F32)
                z[rows, pl.ds(128 * n, 128)] = r[:, :128]
                z[rows, pl.ds(FP + 128 * n, 128)] = r[:, 128:]
            return run

        return [prep, mm(0), mm(1), mm(2)]

    def mid_pieces(k2):
        r0 = pl.multiple_of(k2 * BLK, BLK)
        g0 = pl.multiple_of(k2 * 3 * BLK, BLK)
        st = {}

        def cmul(tab, br, bi):
            t1 = jnp.dot(tab[pl.ds(g0, BLK), :], br.astype(BF16), preferred_element_type=F32)
            t2 = jnp.dot(tab[pl.ds(g0 + BLK, BLK), :], bi.astype(BF16),
                         preferred_element_type=F32)
            t3 = jnp.dot(tab[pl.ds(g0 + 2 * BLK, BLK), :], (br + bi).astype(BF16),
                         preferred_element_type=F32)
            return t1 - t2, t3 - t1 - t2

        def fwd():
            st[0] = cmul(gm, z[pl.ds(r0, BLK), pl.ds(0, FP)], z[pl.ds(r0, BLK), pl.ds(FP, FP)])

        def inv():
            xr, xi = st[0]
            w_r = jnp.concatenate([wfr[j, pl.ds(k2, BLK, stride=NB), :] for j in range(3)], axis=1)
            w_i = jnp.concatenate([wfi[j, pl.ds(k2, BLK, stride=NB), :] for j in range(3)], axis=1)
            yr = xr * w_r - xi * w_i
            yi = xr * w_i + xi * w_r
            ur, ui = cmul(hm, yr, yi)
            z[pl.ds(r0, BLK), pl.ds(0, FP)] = ur
            z[pl.ds(r0, BLK), pl.ds(FP, FP)] = ui

        return [fwd, inv]

    def wprep_load(n):
        src, dst = ((wr, wtr), (wi, wti))[n]
        for b in range(NB):
            dst[b, pl.ds(320, 8), :] = jnp.zeros((8, 128), F32)
            dst[b, pl.ds(0, DF), :] = src[:, pl.ds(BLK * b, BLK)].astype(F32)

    def wprep_piece(n):
        src, dst = ((wtr, wfr), (wti, wfi))[n // 4]
        for b in range(4 * (n % 4), 4 * (n % 4) + 4):
            rows = [src[b, pl.ds(f2, 64, stride=5), :] for f2 in range(5)]
            dst[0, pl.ds(BLK * b, BLK), :] = jnp.concatenate([rows[1], rows[4]], axis=0).T
            dst[1, pl.ds(BLK * b, BLK), :] = jnp.concatenate([rows[2], rows[3]], axis=0).T
            last = jnp.where(sub == 0, src[b, pl.ds(320, 8), :], 0.0)
            dst[2, pl.ds(BLK * b, BLK), :] = jnp.concatenate(
                [rows[0], last, jnp.zeros((56, 128), F32)], axis=0).T

    def radix16_piece(sign, g, j):
        r0 = g * 8
        re = [z[pl.ds(r0 + BLK * b, 8), pl.ds(128 * j, 128)] for b in range(NB)]
        im = [z[pl.ds(r0 + BLK * b, 8), pl.ds(FP + 128 * j, 128)] for b in range(NB)]
        re, im = _fft_list(re, im, sign)
        for b in range(NB):
            z[pl.ds(r0 + BLK * b, 8), pl.ds(128 * j, 128)] = re[b]
            z[pl.ds(r0 + BLK * b, 8), pl.ds(FP + 128 * j, 128)] = im[b]

    def radix16(sign, bouts, extra):
        n = 0
        for g in range(BLK // 8):
            for j in range(FP // 128):
                if n % 6 == 0 and bouts:
                    bout_piece(bouts.pop(0))
                if n % 6 == 3 and extra:
                    wprep_piece(extra.pop(0))
                radix16_piece(sign, g, j)
                n += 1

    def make_qblock(first_half, kw=KW, last=False):
        koff = KW - kw
        row = lax.broadcasted_iota(jnp.int32, (kw, BLK), 0) + koff
        col = lax.broadcasted_iota(jnp.int32, (kw, BLK), 1)

        def qblock(i, carry):
            if first_half:
                xa_copy(i).wait()
                extra = a1_pieces(i)
            else:
                ma = mid_pieces(2 * (i - NB // 2))
                mb = mid_pieces(2 * (i - NB // 2) + 1)
                extra = [ma[0], mb[0], ma[1], mb[1]]

            r0 = pl.multiple_of(i * BLK, BLK)
            q = qnext[...]
            kscr[pl.ds(r0 + WIN, BLK), :] = knext[...]
            vtscr[:, pl.ds(r0 + WIN, BLK)] = vtnext[...]
            todo = [] if last else proj_pieces(i + 1)

            dist = col - row + WIN
            valid = jnp.logical_and(dist >= 0, dist < WIN)
            bias = jnp.where(valid, 0.0, -1e30).astype(F32)

            def scores(grp):
                t0, w, heads = grp
                lane = lax.broadcasted_iota(jnp.int32, (BLK, w), 1) + t0 * 128
                qt = q[:, t0 * 128:t0 * 128 + w]
                qcat = jnp.concatenate(
                    [jnp.where(jnp.logical_and(lane >= DH * hh, lane < DH * hh + DH),
                               qt, jnp.zeros((), BF16)) for hh in heads], axis=0)
                kt = kscr[pl.ds(r0 + koff, kw), t0 * 128:t0 * 128 + w]
                st = lax.dot_general(kt, qcat, (((1,), (1,)), ((), ())),
                                     preferred_element_type=F32)
                bcat = jnp.concatenate([bias] * len(heads), axis=1)
                if kw < KW:
                    st = st + bcat
                else:
                    st = jnp.concatenate(
                        [st[:BLK] + bcat[:BLK], st[BLK:2 * BLK],
                         st[2 * BLK:] + bcat[2 * BLK:]], axis=0)
                return st, jnp.max(st, axis=0, keepdims=True)

            pieces = {}
            st_next = scores(_GROUPS[0])
            for gi, grp in enumerate(_GROUPS):
                st_all, m_all = st_next
                if gi + 1 < len(_GROUPS):
                    st_next = scores(_GROUPS[gi + 1])
                for j, hh in enumerate(grp[2]):
                    p = jnp.exp2(st_all[:, j * BLK:(j + 1) * BLK]
                                 - m_all[:, j * BLK:(j + 1) * BLK])
                    l = jnp.sum(p, axis=0, keepdims=True)
                    a = ((DH * hh) // 16) * 16
                    vth = vtscr[a:a + 32, pl.ds(r0 + koff, kw)]
                    ot = jnp.dot(vth, p.astype(BF16), preferred_element_type=F32)
                    pieces[hh] = ot * (1.0 / l)
                    if hh % 2 == 1 and todo:
                        todo.pop(0)()
                    if hh % 6 == 2 and extra:
                        extra.pop(0)()
            while todo:
                todo.pop(0)()
            while extra:
                extra.pop(0)()
            rows = []
            for g in range(H // 4):
                o0, o1, o2, o3 = (pieces[4 * g + n] for n in range(4))
                rows += [o0[0:16], jnp.where(sub < 4, o0[16:24], o1[0:8]), o1[8:24],
                         o2[8:24], jnp.where(sub < 4, o2[24:32], o3[8:16]), o3[16:32]]
            otscr[:, pl.ds(r0, BLK)] = jnp.concatenate(rows, axis=0).astype(BF16)
            return carry
        return qblock

    first = proj_pieces(0)
    copies[1].wait()
    copies[0].wait()
    for run in first[:5]:
        run()
    copies[10].wait()
    for run in first[5:10]:
        run()
    copies[11].wait()
    wvt[...] = wqkv[:, 2 * D:3 * D].astype(F32).T.astype(BF16)
    for run in first[10:]:
        run()
    copies[3].wait()

    with jax.named_scope('loop1'):
        make_qblock(True, BLK)(0, 0)
        copies[9].wait()
        make_qblock(True, 2 * BLK)(1, 0)
        lax.fori_loop(2, NB // 2, make_qblock(True), 0)

    for n in (2, 4, 5, 6, 7, 8):
        copies[n].wait()
    with jax.named_scope('r16f'):
        wprep_load(0)
        wprep_load(1)
        radix16(-1, list(range(0, NB // 2)), list(range(8)))

    with jax.named_scope('loop2'):
        lax.fori_loop(NB // 2, NB - 1, make_qblock(False), 0)
        make_qblock(False, last=True)(NB - 1, 0)

    with jax.named_scope('r16i'):
        radix16(+1, list(range(NB // 2, NB)), [])

    def a_copy(c):
        return pltpu.make_async_copy(
            astage.at[pl.ds(c * CH, CH), :], out_h.at[pl.ds(c * CH, CH), pl.ds(0, D)],
            osems.at[NCH + c])

    with jax.named_scope('A3'):
        for c in range(NCH):
            rows = pl.ds(c * CH, CH)
            t = []
            for n in range(3):
                y = jnp.concatenate([z[rows, pl.ds(128 * n, 128)],
                                     z[rows, pl.ds(FP + 128 * n, 128)]], axis=1).astype(BF16)
                if n < 2:
                    t.append(jnp.dot(y, mi[pl.ds(256 * n, 256), :], preferred_element_type=F32))
                else:
                    t.append(jnp.dot(y, mi[pl.ds(512, 256), pl.ds(0, 128)],
                                     preferred_element_type=F32))
            p1, q1 = t[0][:, :128], t[0][:, 128:]
            p2, q2 = t[1][:, :128], t[1][:, 128:]
            t0 = t[2]
            e1, o1 = t0 + C1 * p1 + C2 * p2, S1 * q1 + S2 * q2
            e2, o2 = t0 + C2 * p1 + C1 * p2, S2 * q1 - S1 * q2
            astage[rows, :] = jnp.concatenate(
                [t0 + p1 + p2, e1 - o1, e2 - o2, e2 + o2, e1 + o1], axis=1).astype(BF16)
            a_copy(c).start()
    for c in range(NCH):
        out_copy(c).wait()
        a_copy(c).wait()


@jax.jit
def pallas_concat_heads__spectral_gfnet__sliding_block__prompt_kernel(
    A_x: jax.Array,
    A_w_r: jax.Array,
    A_w_i: jax.Array,
    B_x: jax.Array,
    B_wqkv: jax.Array,
    B_wo: jax.Array,
):
    mf, mi, g, h = (jnp.asarray(t, dtype=BF16) for t in _dft_tables())
    xa = A_x.reshape(S, D)
    xb = B_x.reshape(S, D)
    any_spec = pl.BlockSpec(memory_space=pl.ANY)
    out = pl.pallas_call(
        _kernel,
        out_shape=jax.ShapeDtypeStruct((S, 2 * D), BF16),
        in_specs=[any_spec] * 10,
        out_specs=any_spec,
        scratch_shapes=[
            pltpu.VMEM((S, D), BF16),
            pltpu.VMEM((DF, S), BF16),
            pltpu.VMEM((DF, S), BF16),
            pltpu.VMEM((S, D), BF16),
            pltpu.VMEM((D, 3 * D), BF16),
            pltpu.VMEM((D, D), BF16),
            pltpu.VMEM((5 * 128, 256), BF16),
            pltpu.VMEM((6 * 128, 256), BF16),
            pltpu.VMEM((NB * 3 * BLK, BLK), BF16),
            pltpu.VMEM((NB * 3 * BLK, BLK), BF16),
            pltpu.VMEM((S + WIN, D), BF16),
            pltpu.VMEM((D, S + WIN), BF16),
            pltpu.VMEM((D, S), BF16),
            pltpu.VMEM((BLK, D), BF16),
            pltpu.VMEM((BLK, D), BF16),
            pltpu.VMEM((D, BLK), BF16),
            pltpu.VMEM((D, D), BF16),
            pltpu.VMEM((S, 2 * FP), F32),
            pltpu.VMEM((3, S, 128), F32),
            pltpu.VMEM((3, S, 128), F32),
            pltpu.VMEM((NB, 328, 128), F32),
            pltpu.VMEM((NB, 328, 128), F32),
            pltpu.VMEM((S, D), BF16),
            pltpu.VMEM((S, D), BF16),
            pltpu.SemaphoreType.DMA((12,)),
            pltpu.SemaphoreType.DMA((8,)),
            pltpu.SemaphoreType.DMA((16,)),
        ],
        compiler_params=pltpu.CompilerParams(vmem_limit_bytes=120 * 1024 * 1024),
    )(xa, A_w_r.T, A_w_i.T, xb, B_wqkv, B_wo, mf, mi, g, h)
    return out.reshape(1, S, 2 * D)
```
